```python
import jax
import jax.numpy as jnp

def _softmax(x, axis=-1):
    return jax.nn.softmax(x, axis=axis)

def _gelu(x):
    return jax.nn.gelu(x, approximate=True)

def _silu(x):
    return jax.nn.silu(x)

def _sigmoid(x):
    return jax.nn.sigmoid(x)

def _layernorm(x, axis=-1, eps=1e-05):
    m = jnp.mean(x, axis=axis, keepdims=True)
    v = jnp.var(x, axis=axis, keepdims=True)
    return (x - m) / jnp.sqrt(v + eps)

def _scatter_add(tgt, idx, src, axis=0):
    return tgt.at[idx].add(src)

def _segment_sum(src, seg, n):
    return jax.ops.segment_sum(src, seg, n)

class _Rng:

    def __init__(self, key):
        self._k = key

    def _next(self):
        self._k, sub = jax.random.split(self._k)
        return sub

    def normal(self, shape):
        return jax.random.normal(self._next(), shape, dtype=jnp.bfloat16)

    def randint(self, lo, hi, shape):
        return jax.random.randint(self._next(), shape, lo, hi, dtype=jnp.int32)

    def uniform(self, shape, lo=0.0, hi=1.0):
        return jax.random.uniform(self._next(), shape, jnp.bfloat16, lo, hi)

    def permutation(self, n):
        return jax.random.permutation(self._next(), n)
kernel_name = 'adaLN_cond__sliding_block_cached__dense_activation_mish__decode'

def setup_inputs():
    _rng = _Rng(jax.random.key(int.from_bytes(__import__("os").urandom(4), "little")))
    _w = lambda a: (lambda t: t.astype(jnp.bfloat16) if jnp.issubdtype(t.dtype, jnp.floating) else t)(jnp.asarray(a))

    def _A_setup():
        B, Sq, D = (1, 1, 640)
        Hq, Hkv, Sk, Dh = (32, 32, 32768, 192)
        assert Hq % Hkv == 0, (Hq, Hkv)
        return {'x': _w((lambda *s: _rng.normal(s) * 0.05)(B, Sq, D)), 'k_cache': _w((lambda *s: _rng.normal(s) * 0.05)(B, Hkv, Sk, Dh)), 'v_cache': _w((lambda *s: _rng.normal(s) * 0.05)(B, Hkv, Sk, Dh)), 'wq': _w((lambda *s: _rng.normal(s) * 0.05)(D, Hq * Dh) * D ** (-0.5)), 'wo': _w((lambda *s: _rng.normal(s) * 0.05)(Hq * Dh, D) * (Hq * Dh) ** (-0.5))}
    _A_in = _A_setup()

    def _B_setup():
        B, S, D, F = (1, 1, 640, 1536)
        return {'x': _w((lambda *s: _rng.normal(s) * 0.05)(B, S, D)), 'w1': _w((lambda *s: _rng.normal(s) * 0.05)(D, F) * D ** (-0.5)), 'b1': _w((lambda *s: _rng.normal(s) * 0.05)(F)), 'w2': _w((lambda *s: _rng.normal(s) * 0.05)(F, D) * F ** (-0.5))}
    _B_in = _B_setup()
    return {'A_x': _A_in['x'], 'A_k_cache': _A_in['k_cache'], 'A_v_cache': _A_in['v_cache'], 'A_wq': _A_in['wq'], 'A_wo': _A_in['wo'], 'B_x': _B_in['x'], 'B_w1': _B_in['w1'], 'B_b1': _B_in['b1'], 'B_w2': _B_in['w2'], 'c': _w((lambda *s: _rng.normal(s) * 0.05)(1, 640)), 'w_mod': _w((lambda *s: _rng.normal(s) * 0.05)(640, 6 * 640) * 640 ** (-0.5))}

def reference(A_x, A_k_cache, A_v_cache, A_wq, A_wo, B_x, B_w1, B_b1, B_w2, c, w_mod):

    def _A_ref(x, k_cache, v_cache, wq, wo):
        B, Sq, D = x.shape
        Hq, Dh = (32, 192)
        Hkv, Sk = (k_cache.shape[1], k_cache.shape[2])
        W = min(4096, max(256, Sk // 4))
        rep = Hq // Hkv
        q = (lambda x, *d: x.transpose(*d))((x @ wq).reshape(B, Sq, Hq, Dh), 0, 2, 1, 3)
        k = jnp.repeat(k_cache[:, :, Sk - W:, :], rep, axis=1)
        v = jnp.repeat(v_cache[:, :, Sk - W:, :], rep, axis=1)
        scores = jnp.einsum('bhqd,bhkd->bhqk', q, k) * Dh ** (-0.5)
        p = _softmax(scores, axis=-1)
        o = jnp.einsum('bhqk,bhkd->bhqd', p, v)
        return (lambda x, *d: x.transpose(*d))(o, 0, 2, 1, 3).reshape(B, Sq, Hq * Dh) @ wo

    def _B_ref(x, w1, b1, w2):
        h = jnp.einsum('bsd,df->bsf', x, w1) + b1
        sp = jnp.log1p(jnp.exp(-jnp.abs(h))) + jnp.where(h > 0, h, jnp.zeros_like(h))
        act = h * jnp.tanh(sp)
        return jnp.einsum('bsf,fd->bsd', act, w2)
    x = A_x
    mod = (_silu(c) @ w_mod).reshape(c.shape[0], 6, 1, -1)
    sa, ca, ga, sb, cb, gb = (mod[:, 0].copy(), mod[:, 1].copy(), mod[:, 2].copy(), mod[:, 3].copy(), mod[:, 4].copy(), mod[:, 5].copy())
    h = _layernorm(x, axis=-1) * (1 + ca) + sa
    x = x + ga * _A_ref(h, A_k_cache, A_v_cache, A_wq, A_wo)
    h = _layernorm(x, axis=-1) * (1 + cb) + sb
    x = x + gb * _B_ref(h, B_w1, B_b1, B_w2)
    return x
```

```python
import jax
import jax.numpy as jnp
from jax import lax
import jax.experimental.pallas as pl
import jax.experimental.pallas.tpu as pltpu

_HQ, _DH = 32, 192
_EPS = 1e-5
_M = 8
_RING = 2


def _layernorm(x):
    m = jnp.mean(x, axis=-1, keepdims=True)
    d = x - m
    v = jnp.mean(d * d, axis=-1, keepdims=True)
    return d / jnp.sqrt(v + _EPS)


def _dot(a, b):
    return jnp.dot(a, b, preferred_element_type=jnp.float32)


def _dot_nt(a, b):
    return lax.dot_general(a, b, (((1,), (1,)), ((), ())), preferred_element_type=jnp.float32)


def _kernel(x_hbm, k_hbm, v_hbm, wq_hbm, wo_hbm, w1_hbm, b1_hbm, w2_hbm, c_hbm, wmod_hbm,
            o_ref,
            x_v, c_v, b1_v, wmod_v, wq_v, wo_v, w1_v, w2_v, kbuf, vbuf, q_s,
            sem_w, sem_k, sem_v):
    sk = k_hbm.shape[1]
    ring, pw, win = kbuf.shape
    n_pairs = k_hbm.shape[0] // pw
    d = x_v.shape[-1]
    f = w2_v.shape[0]

    def kv_copy(hbm, buf, sem, p, slot):
        row = pl.multiple_of(p * pw, pw)
        return pltpu.make_async_copy(
            hbm.at[pl.ds(row, pw), pl.ds(sk - win, win)], buf.at[slot], sem.at[slot])

    cp_c = pltpu.make_async_copy(c_hbm, c_v, sem_w.at[0])
    cp_x = pltpu.make_async_copy(x_hbm, x_v, sem_w.at[1])
    cp_b1 = pltpu.make_async_copy(b1_hbm, b1_v, sem_w.at[2])
    cp_wmod = pltpu.make_async_copy(wmod_hbm, wmod_v, sem_w.at[3])
    cp_wq = pltpu.make_async_copy(wq_hbm, wq_v, sem_w.at[4])
    cp_wo = pltpu.make_async_copy(wo_hbm, wo_v, sem_w.at[5])
    cp_w1 = pltpu.make_async_copy(w1_hbm, w1_v, sem_w.at[6])
    cp_w2 = pltpu.make_async_copy(w2_hbm, w2_v, sem_w.at[7])

    cp_wmod.start()
    cp_c.start()
    cp_x.start()
    cp_b1.start()
    cp_wq.start()
    cp_wo.start()
    for p in range(ring):
        kv_copy(k_hbm, kbuf, sem_k, p, p).start()
        kv_copy(v_hbm, vbuf, sem_v, p, p).start()

    cp_c.wait()
    c = jnp.broadcast_to(c_v[...].astype(jnp.float32), (_M, d))
    sc = (c * jax.nn.sigmoid(c)).astype(jnp.bfloat16)
    cp_wmod.wait()
    mod = _dot(sc, wmod_v[...])
    sa, ca, ga, sb, cb, gb = (mod[:, i * d:(i + 1) * d] for i in range(6))

    cp_x.wait()
    x = jnp.broadcast_to(x_v[...].astype(jnp.float32), (_M, d))
    h = (_layernorm(x) * (1.0 + ca) + sa).astype(jnp.bfloat16)

    cp_wq.wait()
    row = lax.broadcasted_iota(jnp.int32, (_M, pw), 0)
    col = lax.broadcasted_iota(jnp.int32, (_M, pw), 1)
    own = ((row == 0) & (col < _DH)) | ((row == 1) & (col >= _DH))
    for p in range(n_pairs):
        q_s[p] = jnp.where(own, _dot(h, wq_v[:, p * pw:(p + 1) * pw]), 0.0)

    cp_wo.wait()
    scale = _DH ** -0.5

    def body(p, acc):
        slot = lax.rem(p, ring)
        q = q_s[p].astype(jnp.bfloat16)
        kv_copy(k_hbm, kbuf, sem_k, p, slot).wait()
        s = _dot(q, kbuf[slot]) * scale

        @pl.when(p + ring < n_pairs)
        def _():
            kv_copy(k_hbm, kbuf, sem_k, p + ring, slot).start()

        m = jnp.max(s, axis=-1, keepdims=True)
        e = jnp.exp(s - m)
        l = jnp.sum(e, axis=-1, keepdims=True)
        kv_copy(v_hbm, vbuf, sem_v, p, slot).wait()
        o = _dot_nt(e.astype(jnp.bfloat16), vbuf[slot])

        @pl.when(p + ring < n_pairs)
        def _():
            kv_copy(v_hbm, vbuf, sem_v, p + ring, slot).start()

        @pl.when(p + ring == n_pairs - 1)
        def _():
            cp_w1.start()
            cp_w2.start()

        o = jnp.where(own, o / l, 0.0).astype(jnp.bfloat16)
        r0 = pl.multiple_of(p * pw, pw)
        return acc + _dot(o, wo_v[pl.ds(r0, pw), :])

    acc = lax.fori_loop(0, n_pairs, body, jnp.zeros((_M, d), jnp.float32))
    attn = jnp.broadcast_to(jnp.sum(acc, axis=0, keepdims=True), (_M, d))
    x1 = x + ga * attn
    h2 = (_layernorm(x1) * (1.0 + cb) + sb).astype(jnp.bfloat16)

    cp_b1.wait()
    cp_w1.wait()
    u = _dot(h2, w1_v[...]) + b1_v[...].astype(jnp.float32).reshape(1, f)
    sp = jnp.log1p(jnp.exp(-jnp.abs(u))) + jnp.where(u > 0, u, 0.0)
    act = (u * jnp.tanh(sp)).astype(jnp.bfloat16)
    cp_w2.wait()
    out = x1 + gb * _dot(act, w2_v[...])
    o_ref[...] = out[0:1, :].astype(o_ref.dtype)


@jax.jit
def pallas_adaLN_cond__sliding_block_cached__dense_activation_mish__decode_kernel(
    A_x: jax.Array,
    A_k_cache: jax.Array,
    A_v_cache: jax.Array,
    A_wq: jax.Array,
    A_wo: jax.Array,
    B_x: jax.Array,
    B_w1: jax.Array,
    B_b1: jax.Array,
    B_w2: jax.Array,
    c: jax.Array,
    w_mod: jax.Array,
):
    del B_x
    _, hkv, sk, dh = A_k_cache.shape
    assert A_x.shape[:2] == (1, 1) and (hkv, dh) == (_HQ, _DH)
    d = A_x.shape[-1]
    win = min(4096, max(256, sk // 4))
    kt = jnp.swapaxes(A_k_cache, 2, 3).reshape(hkv * dh, sk)
    vt = jnp.swapaxes(A_v_cache, 2, 3).reshape(hkv * dh, sk)
    bf = jnp.bfloat16
    hbm = pl.BlockSpec(memory_space=pltpu.HBM)
    out = pl.pallas_call(
        _kernel,
        out_shape=jax.ShapeDtypeStruct((1, d), A_x.dtype),
        in_specs=[hbm] * 10,
        out_specs=pl.BlockSpec(memory_space=pltpu.VMEM),
        scratch_shapes=[
            pltpu.VMEM((1, d), bf), pltpu.VMEM((1, d), bf), pltpu.VMEM(B_b1.shape, bf),
            pltpu.VMEM(w_mod.shape, bf), pltpu.VMEM(A_wq.shape, bf), pltpu.VMEM(A_wo.shape, bf),
            pltpu.VMEM(B_w1.shape, bf), pltpu.VMEM(B_w2.shape, bf),
            pltpu.VMEM((_RING, 2 * dh, win), bf), pltpu.VMEM((_RING, 2 * dh, win), bf),
            pltpu.VMEM((hkv // 2, _M, 2 * dh), jnp.float32),
            pltpu.SemaphoreType.DMA((8,)), pltpu.SemaphoreType.DMA((_RING,)),
            pltpu.SemaphoreType.DMA((_RING,)),
        ],
        compiler_params=pltpu.CompilerParams(vmem_limit_bytes=100 * 1024 * 1024),
        name="adaln_decode_block",
    )(A_x.reshape(1, d), kt, vt, A_wq, A_wo, B_w1, B_b1, B_w2, c, w_mod)
    return out.reshape(A_x.shape)
```

```python
import functools

import jax
import jax.numpy as jnp
from jax import lax
import jax.experimental.pallas as pl
import jax.experimental.pallas.tpu as pltpu

_HQ, _DH = 32, 192
_EPS = 1e-5
_M = 8
_L = 128
_PW = 2 * _DH
_T = _PW // _L


def _layernorm(x):
    m = jnp.mean(x, axis=-1, keepdims=True)
    d = x - m
    v = jnp.mean(d * d, axis=-1, keepdims=True)
    return d / jnp.sqrt(v + _EPS)


def _dot(a, b):
    return jnp.dot(a, b, preferred_element_type=jnp.float32)


def _dot_nt(a, b):
    return lax.dot_general(a, b, (((1,), (1,)), ((), ())), preferred_element_type=jnp.float32)


def _div(i, n):
    return i // n if isinstance(i, int) else lax.div(i, n)


def _rem(i, n):
    return i % n if isinstance(i, int) else lax.rem(i, n)


def _hint(i, m):
    return i if isinstance(i, int) else pl.multiple_of(i, m)


class _Run:
    def __init__(self, groups, size, start, wait, step=None, before=None, after=None, first=0):
        self.groups, self.size, self.n, self.first = groups, size, groups * size, first
        self.start, self.wait, self.step, self.before, self.after = start, wait, step, before, after


def make(name="k4", ns=32, d1=12, d0=8, rb=320, g=4, compute=True, nobc=True,
         pm=(8, 8, 768, 1), pq=(10, 8, 512, 2), po=(8, 8, 640, 1), pu=(4, 8, 1536, 1), pd=(3, 32, 640, 1)):
    assert ns & (ns - 1) == 0 and max(d0, d1) + g <= ns

    def kernel(x_hbm, k_hbm, v_hbm, wq_hbm, wo_hbm, w1_hbm, b1_hbm, w2_hbm, c_hbm, wmod_hbm,
               o_ref,
               x_v, c_v, b1_v, wmod_v, wq_v, wo_v, w1_v, w2_v, ring, mod_s, q_s, s_s, act_s, sem_in, sem):
        sk = k_hbm.shape[1]
        d = x_v.shape[-1]
        f = b1_v.shape[0]
        n_pairs = k_hbm.shape[0] // _PW
        nblk = s_s.shape[0]
        win = nblk * _L
        scale = _DH ** -0.5

        def window(src, p):
            def start(i, slot, prio):
                lo, n = (0, rb) if prio else (rb, _PW - rb)
                pltpu.make_async_copy(
                    src.at[pl.ds(_hint(p * _PW + lo, 16), n), pl.ds(_hint(sk - win + i * _L, _L), _L)],
                    ring.at[slot, pl.ds(lo, n)], sem.at[slot]).start(priority=prio)

            def wait(_, slot):
                pltpu.make_async_copy(ring.at[slot], ring.at[slot], sem.at[slot]).wait()

            return start, wait

        def weight(src, dst, h, w, a):
            bands, nrow, ncol = src.shape
            nc = ncol // w

            def patch(i):
                return pl.ds(_hint(_div(i, nc) * h, h), h), pl.ds(_hint(_rem(i, nc) * w, w), w)

            def start(i, slot, prio):
                idx = (pl.ds(0, bands - a) if prio else pl.ds(bands - a, a), *patch(i))
                pltpu.make_async_copy(src.at[idx], dst.at[idx], sem.at[slot]).start(priority=prio)

            def wait(i, slot):
                whole = dst.at[(slice(None), *patch(i))]
                pltpu.make_async_copy(whole, whole, sem.at[slot]).wait()

            return (nrow // h) * nc, start, wait

        def locate(runs, pos):
            for r in runs:
                if pos < r.n:
                    return r, pos
                pos -= r.n
            return None, 0

        def stream(runs, t0, ahead):
            total = sum(r.n for r in runs)

            def targets(pos):
                if pos < total:
                    return [(None, *locate(runs, pos))]
                found = [(cond, *locate(rs, pos - total)) for cond, rs in ahead]
                return [t for t in found if t[1] is not None]

            def follows(a, b, size):
                flat = lambda plan: [t for step in plan for tgts in step for t in tgts + [None]]
                a, b = flat(a), flat(b)
                return len(a) == len(b) and all(
                    (x is None and y is None)
                    or (x is not None and y is not None and x[1] is y[1] and y[2] == x[2] + size)
                    for x, y in zip(a, b))

            base = 0
            for run in runs:
                plans = [[[targets(base + grp * run.size + i + dist) for dist in (d1, d0)]
                          for i in range(run.size)] for grp in range(run.groups)]
                carry = run.before() if (run.before and compute) else None
                g0 = 0
                while g0 < run.groups:
                    g1 = g0 + 1
                    while g1 < run.groups and follows(plans[g1 - 1], plans[g1], run.size):
                        g1 += 1

                    def body(j, carry, g0=g0, run=run, base=base):
                        i0 = (g0 + j) * run.size
                        t = t0 + base + i0
                        for i, step in enumerate(plans[g0]):
                            run.wait(run.first + i0 + i, (t + i) & (ns - 1))
                            for prio, dist, tgts in zip((1, 0), (d1, d0), step):
                                for cond, nxt, k in tgts:
                                    go = functools.partial(
                                        nxt.start, nxt.first + k + j * run.size, (t + i + dist) & (ns - 1), prio)
                                    go() if cond is None else pl.when(cond)(go)
                        if not compute or run.step is None:
                            return carry
                        return run.step(g0 + j, [(t + i) & (ns - 1) for i in range(run.size)], carry)

                    carry = body(0, carry) if g1 - g0 == 1 else lax.fori_loop(0, g1 - g0, body, carry)
                    g0 = g1
                if run.after and compute:
                    run.after(carry)
                base += run.n

        def cols(ref, grp):
            return ref[:, :, pl.ds(_hint(grp * _PW, _PW), _PW)].reshape(d, _PW)

        def mod(i):
            flat = jnp.concatenate([mod_s[j] for j in range(mod_s.shape[0])], axis=1)
            return flat[:, i * d:(i + 1) * d]

        def rows(ref):
            return jnp.broadcast_to(ref[...].astype(jnp.float32), (_M, d))

        def own():
            row = lax.broadcasted_iota(jnp.int32, (_M, _PW), 0)
            col = lax.broadcasted_iota(jnp.int32, (_M, _PW), 1)
            return ((row == 0) & (col < _DH)) | ((row == 1) & (col >= _DH))

        def pair_runs(p, state):
            def k_before():
                state["q"] = q_s[p].astype(jnp.bfloat16)
                return jnp.full((_M, _L), -jnp.inf, jnp.float32)

            def k_step(grp, slots, m):
                for i, slot in enumerate(slots):
                    s = _dot(state["q"], ring[slot]) * scale
                    s_s[grp * g + i] = s
                    m = jnp.maximum(m, s)
                return m

            def k_done(m):
                state["m"] = jnp.broadcast_to(jnp.max(m, axis=-1, keepdims=True), (_M, _L))

            def v_step(grp, slots, carry):
                l, acc = carry[0], list(carry[1:])
                for i, slot in enumerate(slots):
                    e = jnp.exp(s_s[grp * g + i] - state["m"])
                    l = l + e
                    eb = e.astype(jnp.bfloat16)
                    for t in range(_T):
                        acc[t] = acc[t] + _dot_nt(eb, ring[slot, pl.ds(t * _L, _L), :])
                return (l, *acc)

            def v_done(carry):
                l = jnp.sum(carry[0], axis=-1, keepdims=True)
                o = jnp.concatenate(carry[1:], axis=1) / l
                o = jnp.where(own(), o, 0.0).astype(jnp.bfloat16)
                per = wo_v.shape[1] // _PW
                wo = wo_v[_div(p, per), pl.ds(_hint(_rem(p, per) * _PW, _PW), _PW), :]
                state["attn"] = state["attn"] + _dot(o, wo)

            return [
                _Run(nblk // g, g, *window(k_hbm, p), k_step, k_before, k_done),
                _Run(nblk // g, g, *window(v_hbm, p), v_step,
                     lambda: (jnp.zeros((_M, _L), jnp.float32),) * (1 + _T), v_done),
            ]

        small = [pltpu.make_async_copy(s, t, sem_in.at[i])
                 for i, (s, t) in enumerate(((c_hbm, c_v), (x_hbm, x_v), (b1_hbm, b1_v)))]
        top = {}

        def mod_before():
            small[0].wait()
            c = rows(c_v)
            top["sc"] = (c * jax.nn.sigmoid(c)).astype(jnp.bfloat16)

        def mod_step(grp, _, carry):
            mod_s[grp] = _dot(top["sc"], cols(wmod_v, grp))
            return carry

        def mod_done(_):
            small[1].wait()
            top["h"] = (_layernorm(rows(x_v)) * (1.0 + mod(1)) + mod(0)).astype(jnp.bfloat16)

        def q_step(grp, _, carry):
            q_s[grp] = jnp.where(own(), _dot(top["h"], cols(wq_v, grp)), 0.0)
            return carry

        def norm2():
            attn = jnp.broadcast_to(jnp.sum(top["attn"], axis=0, keepdims=True), (_M, d))
            top["x"] = rows(x_v) + mod(2) * attn
            top["h"] = (_layernorm(top["x"]) * (1.0 + mod(4)) + mod(3)).astype(jnp.bfloat16)
            small[2].wait()
            b1 = b1_v[...].astype(jnp.float32).reshape(1, f)
            for grp in range(f // _PW):
                act_s[grp] = jnp.broadcast_to(b1[:, grp * _PW:(grp + 1) * _PW], (_M, _PW))

        def up(grp):
            u = _dot(top["h"], cols(w1_v, grp)) + act_s[grp]
            sp = jnp.log1p(jnp.exp(-jnp.abs(u))) + jnp.where(u > 0, u, 0.0)
            act_s[grp] = u * jnp.tanh(sp)

        def down(j, y):
            per = w2_v.shape[1] // _L
            for b in range(w2_v.shape[0]):
                tile = b * per + j
                a = act_s[tile // _T][:, (tile % _T) * _L:(tile % _T + 1) * _L].astype(jnp.bfloat16)
                y = y + _dot(a, w2_v[b, pl.ds(j * _L, _L), :])
            return y

        n_m, *io_m = weight(wmod_hbm, wmod_v, *pm[1:])
        n_q, *io_q = weight(wq_hbm, wq_v, *pq[1:])
        n_o, *io_o = weight(wo_hbm, wo_v, *po[1:])
        n_u, *io_u = weight(w1_hbm, w1_v, *pu[1:])
        n_d, *io_d = weight(w2_hbm, w2_v, *pd[1:])
        n_mod = mod_s.shape[0]
        sz = n_q // (n_mod + 1)
        head = [
            _Run(n_m, 1, *io_m),
            _Run(n_mod, sz, *io_q, mod_step, mod_before, mod_done),
            _Run(n_q - n_mod * sz, 1, *io_q, first=n_mod * sz),
            _Run(n_pairs, n_o // n_pairs, *io_o, q_step),
        ]
        assert n_o % n_pairs == 0
        n_up, n_down = f // _PW, w2_v.shape[1] // _L
        per_down = n_d // n_down
        assert per_down >= n_up
        top["y"] = jnp.zeros((_M, d), jnp.float32) if compute else None

        def down_step(j):
            def step(grp, _, carry):
                top["y"] = down(j, top["y"])
                return carry
            return step

        tail = [
            _Run(n_u, 1, *io_u, None, norm2),
            _Run(n_up, 1, *io_d, lambda grp, _, carry: up(grp)),
            *([_Run(1, per_down - n_up, *io_d, first=n_up)] if per_down > n_up else []),
            _Run(1, 1, *io_d, down_step(0), first=per_down),
            _Run(1, per_down - 1, *io_d, down_step(1), first=per_down + 1),
            *[_Run(1, per_down, *io_d, down_step(j), first=j * per_down) for j in range(2, n_down)],
        ]

        head[0].start(0, 0, 1)
        for cp in small:
            cp.start()
        for t in range(max(d0, d1)):
            if 0 < t < d1:
                head[0].start(t, t, 1)
            if t < d0:
                head[0].start(t, t, 0)
        stream(head, 0, [(None, pair_runs(0, {}))])
        n_head = sum(r.n for r in head)

        def pair(p, attn):
            state = dict(attn=attn)
            stream(pair_runs(p, state), n_head + p * 2 * nblk,
                   [(p + 1 < n_pairs, pair_runs(p + 1, {})), (p + 1 == n_pairs, tail)])
            return state["attn"]

        top["attn"] = lax.fori_loop(0, n_pairs, pair, jnp.zeros((_M, d), jnp.float32))
        stream(tail, n_head + n_pairs * 2 * nblk, [])
        if compute:
            o_ref[...] = (top["x"] + mod(5) * top["y"])[0:1, :].astype(o_ref.dtype)
        else:
            for cp in small:
                cp.wait()
            o_ref[...] = x_v[...]

    def fn(A_x, A_k_cache, A_v_cache, A_wq, A_wo, B_x, B_w1, B_b1, B_w2, c, w_mod):
        del B_x
        _, hkv, sk, dh = A_k_cache.shape
        d = A_x.shape[-1]
        f = B_w1.shape[1]
        win = min(4096, max(256, sk // 4))
        kt = jnp.swapaxes(A_k_cache, 2, 3).reshape(hkv * dh, sk)
        vt = jnp.swapaxes(A_v_cache, 2, 3).reshape(hkv * dh, sk)
        band = lambda w, n: w.reshape(n, w.shape[0] // n, w.shape[1])
        wm, wq, wo, w1, w2 = (band(w, p[0]) for w, p in
                              ((w_mod, pm), (A_wq, pq), (A_wo, po), (B_w1, pu), (B_w2, pd)))
        bf, f32 = jnp.bfloat16, jnp.float32
        hbm = pl.BlockSpec(memory_space=pltpu.HBM)
        out = pl.pallas_call(
            kernel,
            out_shape=jax.ShapeDtypeStruct((1, d), A_x.dtype),
            in_specs=[hbm] * 10,
            out_specs=pl.BlockSpec(memory_space=pltpu.VMEM),
            scratch_shapes=[
                pltpu.VMEM((1, d), bf), pltpu.VMEM((1, d), bf), pltpu.VMEM(B_b1.shape, bf),
                *[pltpu.VMEM(w.shape, bf) for w in (wm, wq, wo, w1, w2)],
                pltpu.VMEM((ns, _PW, _L), bf),
                pltpu.VMEM((w_mod.shape[1] // _PW, _M, _PW), f32),
                pltpu.VMEM((hkv // 2, _M, _PW), f32),
                pltpu.VMEM((win // _L, _M, _L), f32),
                pltpu.VMEM((f // _PW, _M, _PW), f32),
                pltpu.SemaphoreType.DMA((3,)), pltpu.SemaphoreType.DMA((ns,)),
            ],
            compiler_params=pltpu.CompilerParams(disable_bounds_checks=nobc, vmem_limit_bytes=48 * 1024 * 1024),
            name=name,
        )(A_x.reshape(1, d), kt, vt, wq, wo, w1, B_b1, w2, c, wm)
        return out.reshape(A_x.shape)

    return fn


_impl = make(name="adaln_decode_block", g=2)


@jax.jit
def pallas_adaLN_cond__sliding_block_cached__dense_activation_mish__decode_kernel(
    A_x, A_k_cache, A_v_cache, A_wq, A_wo, B_x, B_w1, B_b1, B_w2, c, w_mod
):
    return _impl(A_x, A_k_cache, A_v_cache, A_wq, A_wo, B_x, B_w1, B_b1, B_w2, c, w_mod)
```

```python
import functools

import jax
import jax.numpy as jnp
from jax import lax
import jax.experimental.pallas as pl
import jax.experimental.pallas.tpu as pltpu

_HQ, _DH = 32, 192
_EPS = 1e-5
_M = 8
_L = 128
_PW = 2 * _DH
_T = _PW // _L

_SEMS = 32
_MAIN, _SLIVER = 1, 0
_AHEAD = {_MAIN: 26, _SLIVER: 18}
_PARTS = 2
_KV_SLIVER = 16
_GROUP = 4

_MOD_PATCH = (8, 8, 384)
_Q_PATCH = (10, 8, 256)
_O_PATCH = (8, 8, 640)
_UP_PATCH = (4, 8, 768)
_DOWN_PATCH = (3, 16, 640)


def _layernorm(x):
    m = jnp.mean(x, axis=-1, keepdims=True)
    d = x - m
    v = jnp.mean(d * d, axis=-1, keepdims=True)
    return d / jnp.sqrt(v + _EPS)


def _dot(a, b):
    return jnp.dot(a, b, preferred_element_type=jnp.float32)


def _dot_nt(a, b):
    return lax.dot_general(a, b, (((1,), (1,)), ((), ())), preferred_element_type=jnp.float32)


def _hint(i, m):
    return i if isinstance(i, int) else pl.multiple_of(i, m)


class _Source:
    def __init__(self, n, period, start, wait):
        self.n, self.period, self.start, self.wait = n, period, start, wait


class _Run:
    def __init__(self, source, groups, size, step=None, before=None, after=None, first=0):
        self.source, self.groups, self.size, self.first = source, groups, size, first
        self.n = groups * size
        self.step, self.before, self.after = step, before, after


def _locate(runs, pos):
    for run in runs:
        if pos < run.n:
            return run.source, run.first + pos
        pos -= run.n
    return None, 0


def _stream(runs, t0, following, sems):
    total = sum(run.n for run in runs)

    def at(pos):
        if pos < total:
            return [(None, *_locate(runs, pos))]
        found = [(cond, *_locate(later, pos - total)) for cond, later in following]
        return [x for x in found if x[1] is not None]

    def repeats(a, b, size):
        a, b = ([x for entry in plan for alts in entry for x in alts + [None]] for plan in (a, b))
        return len(a) == len(b) and all(
            x is y if None in (x, y)
            else x[1] is y[1] and y[2] == x[2] + size and size % x[1].period == 0
            for x, y in zip(a, b))

    def sem(t):
        return sems.at[t & (_SEMS - 1)]

    base = 0
    for run in runs:
        plans = [[[at(base + grp * run.size + i + dist) for dist in (0, *_AHEAD.values())]
                  for i in range(run.size)] for grp in range(run.groups)]
        carry = run.before() if run.before else None
        lo = 0
        while lo < run.groups:
            hi = lo + 1
            while hi < run.groups and repeats(plans[hi - 1], plans[hi], run.size):
                hi += 1

            def group(j, carry, lo=lo, run=run, base=base):
                def index(source, k):
                    return k // source.period + j * (run.size // source.period), k % source.period

                t = t0 + base + (lo + j) * run.size
                for i, ([(_, source, k)], *later) in enumerate(plans[lo]):
                    source.wait(*index(source, k), sem(t + i))
                    for (priority, dist), alts in zip(_AHEAD.items(), later):
                        for cond, source, k in alts:
                            start = functools.partial(
                                source.start, *index(source, k), sem(t + i + dist), priority)
                            if cond is None:
                                start()
                            else:
                                pl.when(cond)(start)
                return run.step(lo + j, carry) if run.step else carry

            carry = group(0, carry) if hi - lo == 1 else lax.fori_loop(0, hi - lo, group, carry)
            lo = hi
        if run.after:
            run.after(carry)
        base += run.n


def _weight_source(src, dst, h, w):
    bands, nrow, ncol = src.shape

    def patch(r, c):
        return pl.ds(_hint(r * h, h), h), pl.ds(c * w, w)

    def start(r, c, sem, priority):
        idx = (pl.ds(0, bands - 1) if priority == _MAIN else pl.ds(bands - 1, 1), *patch(r, c))
        pltpu.make_async_copy(src.at[idx], dst.at[idx], sem).start(priority=priority)

    def wait(r, c, sem):
        both = dst.at[(slice(None), *patch(r, c))]
        pltpu.make_async_copy(both, both, sem).wait()

    return _Source((nrow // h) * (ncol // w), ncol // w, start, wait)


def _window_source(src, dst, pair):
    nblk = dst.shape[0]
    first = src.shape[1] - nblk * _L
    h = _PW // _PARTS

    def start(blk, part, sem, priority):
        lo, n = ((part * h, h - _KV_SLIVER) if priority == _MAIN
                 else ((part + 1) * h - _KV_SLIVER, _KV_SLIVER))
        pltpu.make_async_copy(
            src.at[pl.ds(_hint(pair * _PW + lo, 16), n), pl.ds(_hint(first + blk * _L, _L), _L)],
            dst.at[blk, pl.ds(lo, n)], sem).start(priority=priority)

    def wait(blk, part, sem):
        both = dst.at[blk, pl.ds(part * h, h)]
        pltpu.make_async_copy(both, both, sem).wait()

    return _Source(nblk * _PARTS, _PARTS, start, wait)


def _kernel(x_hbm, k_hbm, v_hbm, wq_hbm, wo_hbm, w1_hbm, b1_hbm, w2_hbm, c_hbm, wmod_hbm,
            o_ref,
            x_v, c_v, b1_v, wmod_v, wq_v, wo_v, w1_v, w2_v, kv_v,
            mod_s, q_s, score_s, act_s, col_s, small_sems, sems):
    d = x_v.shape[-1]
    f = b1_v.shape[0]
    n_pairs = k_hbm.shape[0] // _PW
    nblk = kv_v.shape[0]
    scale = _DH ** -0.5
    assert max(_AHEAD.values()) + _PARTS * _GROUP <= _PARTS * nblk
    assert max(_AHEAD.values()) < _SEMS

    small = [pltpu.make_async_copy(src, dst, small_sems.at[i])
             for i, (src, dst) in enumerate(((c_hbm, c_v), (x_hbm, x_v), (b1_hbm, b1_v)))]
    val = {}

    def rows(ref):
        return jnp.broadcast_to(ref[...].astype(jnp.float32), (_M, d))

    def cols(ref, i, w):
        return ref[:, :, pl.ds(_hint(i * w, _L), w)].reshape(d, w)

    def per_head(y):
        row = lax.broadcasted_iota(jnp.int32, y.shape, 0)
        col = lax.broadcasted_iota(jnp.int32, y.shape, 1)
        return jnp.where(((row == 0) & (col < _DH)) | ((row == 1) & (col >= _DH)), y, 0.0)

    def condition():
        small[0].wait()
        c = rows(c_v)
        val["c"] = (c * jax.nn.sigmoid(c)).astype(jnp.bfloat16)

    def modulate(i, carry):
        mod_s[i] = _dot(val["c"], cols(wmod_v, i, d))
        return carry

    def norm_a(_):
        small[1].wait()
        val["h"] = (_layernorm(rows(x_v)) * (1.0 + mod_s[1]) + mod_s[0]).astype(jnp.bfloat16)

    def query(pair, carry):
        q_s[pair] = per_head(_dot(val["h"], cols(wq_v, pair, _PW)))
        return carry

    def attention_runs(pair):
        def load_query():
            val["q"] = q_s[pair].astype(jnp.bfloat16)
            return jnp.full((_M, _L), -jnp.inf, jnp.float32)

        def scores(grp, top):
            for blk in (grp * _GROUP + i for i in range(_GROUP)):
                s = _dot(val["q"], kv_v[blk]) * scale
                score_s[blk] = s
                top = jnp.maximum(top, s)
            return top

        def row_max(top):
            val["max"] = jnp.broadcast_to(jnp.max(top, axis=-1, keepdims=True), (_M, _L))

        def values(grp, carry):
            total, *acc = carry
            for blk in (grp * _GROUP + i for i in range(_GROUP)):
                e = jnp.exp(score_s[blk] - val["max"])
                total = total + e
                e = e.astype(jnp.bfloat16)
                acc = [acc[t] + _dot_nt(e, kv_v[blk, pl.ds(t * _L, _L), :]) for t in range(_T)]
            return (total, *acc)

        def project(carry):
            total, *acc = carry
            o = jnp.concatenate(acc, axis=1) / jnp.sum(total, axis=-1, keepdims=True)
            per_band = wo_v.shape[1] // _PW
            row = _hint(lax.rem(pair, per_band) * _PW, _PW)
            wo = wo_v[lax.div(pair, per_band), pl.ds(row, _PW), :]
            val["attn"] = val["attn"] + _dot(per_head(o).astype(jnp.bfloat16), wo)

        def zeros():
            return (jnp.zeros((_M, _L), jnp.float32),) * (1 + _T)

        shape = (nblk // _GROUP, _GROUP * _PARTS)
        return [_Run(_window_source(k_hbm, kv_v, pair), *shape, scores, load_query, row_max),
                _Run(_window_source(v_hbm, kv_v, pair), *shape, values, zeros, project)]

    def norm_b(_):
        attn = jnp.broadcast_to(jnp.sum(val["attn"], axis=0, keepdims=True), (_M, d))
        val["x"] = rows(x_v) + mod_s[2] * attn
        val["h"] = (_layernorm(val["x"]) * (1.0 + mod_s[4]) + mod_s[3]).astype(jnp.bfloat16)
        val["y"] = jnp.zeros((_M, d), jnp.float32)
        small[2].wait()
        b1 = b1_v[...].astype(jnp.float32).reshape(1, f)
        for i in range(f // _PW):
            act_s[i] = jnp.broadcast_to(b1[:, i * _PW:(i + 1) * _PW], (_M, _PW))

    def up(i, carry):
        u = _dot(val["h"], cols(w1_v, i, _PW)) + act_s[i]
        softplus = jnp.log1p(jnp.exp(-jnp.abs(u))) + jnp.where(u > 0, u, 0.0)
        act_s[i] = u * jnp.tanh(softplus)
        return carry

    bands, band_rows, _ = w2_v.shape

    def act(band, j):
        at = band * band_rows + j * _L
        return act_s[at // _PW][:, at % _PW:at % _PW + _L].astype(jnp.bfloat16)

    def down(j, _, carry):
        for band in range(bands):
            val["y"] = val["y"] + _dot(act(band, j), w2_v[band, pl.ds(j * _L, _L), :])
        return carry

    last = band_rows // _L - 1
    h_down = _DOWN_PATCH[1]

    def last_columns():
        for band in range(bands):
            a = act(band, last)[0:1].astype(jnp.float32)
            col_s[band] = jnp.broadcast_to(a, (_L, _L)).T
        return jnp.zeros((_M, d), jnp.float32)

    def down_last(i, acc):
        for band in range(bands):
            w = w2_v[band, pl.ds(_hint(last * _L + i * h_down, h_down), h_down), :]
            a = col_s[band, pl.ds(_hint(i * h_down, h_down), h_down), :]
            prod = w.astype(jnp.float32) * jnp.concatenate([a] * (d // _L), axis=1)
            for r in range(0, h_down, _M):
                acc = acc + prod[r:r + _M]
        return acc

    def finish(acc):
        y = val["y"][0:1] + jnp.sum(acc, axis=0, keepdims=True)
        o_ref[...] = (val["x"][0:1] + mod_s[5, 0:1] * y).astype(o_ref.dtype)

    src_mod = _weight_source(wmod_hbm, wmod_v, *_MOD_PATCH[1:])
    src_q = _weight_source(wq_hbm, wq_v, *_Q_PATCH[1:])
    src_o = _weight_source(wo_hbm, wo_v, *_O_PATCH[1:])
    src_up = _weight_source(w1_hbm, w1_v, *_UP_PATCH[1:])
    src_down = _weight_source(w2_hbm, w2_v, *_DOWN_PATCH[1:])

    n_mod, n_up, per_tile = mod_s.shape[0], f // _PW, _L // h_down
    head = [
        _Run(src_mod, src_mod.n // src_mod.period, src_mod.period),
        _Run(src_q, n_mod, src_q.period, modulate, condition),
        _Run(src_q, src_q.n // src_q.period - n_mod, src_q.period, after=norm_a,
             first=n_mod * src_q.period),
        _Run(src_o, n_pairs, src_o.n // n_pairs, query),
    ]
    tail = [
        _Run(src_up, src_up.n // src_up.period, src_up.period, after=norm_b),
        _Run(src_down, n_up, 1, up),
        _Run(src_down, 1, per_tile - n_up, functools.partial(down, 0), first=n_up),
        *[_Run(src_down, 1, per_tile, functools.partial(down, j), first=j * per_tile)
          for j in range(1, last)],
        _Run(src_down, per_tile, 1, down_last, last_columns, finish, first=last * per_tile),
    ]
    n_head = sum(run.n for run in head)
    assert n_head == src_mod.n + src_q.n + src_o.n
    assert sum(run.n for run in tail) == src_up.n + src_down.n

    for t in range(max(_AHEAD.values())):
        for priority, dist in _AHEAD.items():
            if t < dist:
                src_mod.start(t // src_mod.period, t % src_mod.period, sems.at[t], priority)
        if t == 0:
            for copy in small:
                copy.start()
    _stream(head, 0, [(None, attention_runs(0))], sems)

    per_pair = 2 * nblk * _PARTS

    def attend(pair, attn):
        val["attn"] = attn
        following = [(pair + 1 < n_pairs, attention_runs(pair + 1)), (pair + 1 == n_pairs, tail)]
        _stream(attention_runs(pair), n_head + pair * per_pair, following, sems)
        return val["attn"]

    val["attn"] = lax.fori_loop(0, n_pairs, attend, jnp.zeros((_M, d), jnp.float32))
    _stream(tail, n_head + n_pairs * per_pair, [], sems)


@jax.jit
def pallas_adaLN_cond__sliding_block_cached__dense_activation_mish__decode_kernel(
    A_x: jax.Array,
    A_k_cache: jax.Array,
    A_v_cache: jax.Array,
    A_wq: jax.Array,
    A_wo: jax.Array,
    B_x: jax.Array,
    B_w1: jax.Array,
    B_b1: jax.Array,
    B_w2: jax.Array,
    c: jax.Array,
    w_mod: jax.Array,
):
    del B_x
    _, hkv, sk, dh = A_k_cache.shape
    assert A_x.shape[:2] == (1, 1) and (hkv, dh) == (_HQ, _DH)
    d = A_x.shape[-1]
    f = B_w1.shape[1]
    win = min(4096, max(256, sk // 4))
    kt = jnp.swapaxes(A_k_cache, 2, 3).reshape(hkv * dh, sk)
    vt = jnp.swapaxes(A_v_cache, 2, 3).reshape(hkv * dh, sk)
    wmod, wq, wo, w1, w2 = (
        w.reshape(bands, w.shape[0] // bands, w.shape[1]) for w, (bands, _, _) in (
            (w_mod, _MOD_PATCH), (A_wq, _Q_PATCH), (A_wo, _O_PATCH), (B_w1, _UP_PATCH),
            (B_w2, _DOWN_PATCH)))
    x = A_x.reshape(1, d)
    f32 = jnp.float32
    out = pl.pallas_call(
        _kernel,
        out_shape=jax.ShapeDtypeStruct(x.shape, x.dtype),
        in_specs=[pl.BlockSpec(memory_space=pltpu.HBM)] * 10,
        out_specs=pl.BlockSpec(memory_space=pltpu.VMEM),
        scratch_shapes=[
            *[pltpu.VMEM(a.shape, a.dtype) for a in (x, c, B_b1, wmod, wq, wo, w1, w2)],
            pltpu.VMEM((win // _L, _PW, _L), kt.dtype),
            pltpu.VMEM((w_mod.shape[1] // d, _M, d), f32),
            pltpu.VMEM((hkv // 2, _M, _PW), f32),
            pltpu.VMEM((win // _L, _M, _L), f32),
            pltpu.VMEM((f // _PW, _M, _PW), f32),
            pltpu.VMEM((w2.shape[0], _L, _L), f32),
            pltpu.SemaphoreType.DMA((3,)),
            pltpu.SemaphoreType.DMA((_SEMS,)),
        ],
        compiler_params=pltpu.CompilerParams(
            vmem_limit_bytes=48 * 1024 * 1024,
            disable_semaphore_checks=True,
        ),
        name="adaln_decode_block",
    )(x, kt, vt, wq, wo, w1, B_b1, w2, c, wmod)
    return out.reshape(A_x.shape)
```

```python
import functools

import jax
import jax.numpy as jnp
from jax import lax
import jax.experimental.pallas as pl
import jax.experimental.pallas.tpu as pltpu

_HQ, _DH = 32, 192
_EPS = 1e-5
_M = 8
_L = 128
_PW = 2 * _DH
_T = _PW // _L

_SEMS = 32
_MAIN, _SLIVER = 1, 0
_AHEAD = {_MAIN: 26, _SLIVER: 16}
_PARTS = 2
_KV_SLIVER = 16
_GROUP = 4

_MOD_PATCH = (8, 8, 384)
_Q_PATCH = (10, 8, 256)
_O_PATCH = (8, 8, 640)
_UP_PATCH = (4, 8, 768)
_DOWN_PATCH = (3, 16, 640)


def _layernorm(x):
    m = jnp.mean(x, axis=-1, keepdims=True)
    d = x - m
    v = jnp.mean(d * d, axis=-1, keepdims=True)
    return d / jnp.sqrt(v + _EPS)


def _dot(a, b):
    return jnp.dot(a, b, preferred_element_type=jnp.float32)


def _dot_nt(a, b):
    return lax.dot_general(a, b, (((1,), (1,)), ((), ())), preferred_element_type=jnp.float32)


def _hint(i, m):
    return i if isinstance(i, int) else pl.multiple_of(i, m)


class _Source:
    def __init__(self, n, period, start, wait):
        self.n, self.period, self.start, self.wait = n, period, start, wait


class _Run:
    def __init__(self, source, groups, size, step=None, before=None, after=None, first=0):
        self.source, self.groups, self.size, self.first = source, groups, size, first
        self.n = groups * size
        self.step, self.before, self.after = step, before, after


def _locate(runs, pos):
    for run in runs:
        if pos < run.n:
            return run.source, run.first + pos
        pos -= run.n
    return None, 0


def _stream(runs, t0, following, sems):
    total = sum(run.n for run in runs)

    def at(pos):
        if pos < total:
            return [(None, *_locate(runs, pos))]
        found = [(cond, *_locate(later, pos - total)) for cond, later in following]
        return [x for x in found if x[1] is not None]

    def repeats(a, b, size):
        a, b = ([x for entry in plan for alts in entry for x in alts + [None]] for plan in (a, b))
        return len(a) == len(b) and all(
            x is y if None in (x, y)
            else x[1] is y[1] and y[2] == x[2] + size and size % x[1].period == 0
            for x, y in zip(a, b))

    def sem(t):
        return sems.at[t & (_SEMS - 1)]

    base = 0
    for run in runs:
        plans = [[[at(base + grp * run.size + i + dist) for dist in (0, *_AHEAD.values())]
                  for i in range(run.size)] for grp in range(run.groups)]
        carry = run.before() if run.before else None
        lo = 0
        while lo < run.groups:
            hi = lo + 1
            while hi < run.groups and repeats(plans[hi - 1], plans[hi], run.size):
                hi += 1

            def group(j, carry, lo=lo, run=run, base=base):
                def index(source, k):
                    return k // source.period + j * (run.size // source.period), k % source.period

                t = t0 + base + (lo + j) * run.size
                for i, ([(_, source, k)], *later) in enumerate(plans[lo]):
                    source.wait(*index(source, k), sem(t + i))
                    for (priority, dist), alts in zip(_AHEAD.items(), later):
                        for cond, source, k in alts:
                            start = functools.partial(
                                source.start, *index(source, k), sem(t + i + dist), priority)
                            if cond is None:
                                start()
                            else:
                                pl.when(cond)(start)
                return run.step(lo + j, carry) if run.step else carry

            carry = group(0, carry) if hi - lo == 1 else lax.fori_loop(0, hi - lo, group, carry)
            lo = hi
        if run.after:
            run.after(carry)
        base += run.n


def _weight_source(src, dst, h, w):
    bands, nrow, ncol = src.shape

    def patch(r, c):
        return pl.ds(_hint(r * h, h), h), pl.ds(c * w, w)

    def start(r, c, sem, priority):
        idx = (pl.ds(0, bands - 1) if priority == _MAIN else pl.ds(bands - 1, 1), *patch(r, c))
        pltpu.make_async_copy(src.at[idx], dst.at[idx], sem).start(priority=priority)

    def wait(r, c, sem):
        both = dst.at[(slice(None), *patch(r, c))]
        pltpu.make_async_copy(both, both, sem).wait()

    return _Source((nrow // h) * (ncol // w), ncol // w, start, wait)


def _window_source(src, dst, pair):
    nblk = dst.shape[0]
    first = src.shape[1] - nblk * _L
    spans = {_MAIN: ((_KV_SLIVER, _DH - _KV_SLIVER), (_DH, _DH - _KV_SLIVER)),
             _SLIVER: ((0, _KV_SLIVER), (_PW - _KV_SLIVER, _KV_SLIVER))}

    def start(blk, part, sem, priority):
        lo, n = spans[priority][part]
        pltpu.make_async_copy(
            src.at[pl.ds(_hint(pair * _PW + lo, 16), n), pl.ds(_hint(first + blk * _L, _L), _L)],
            dst.at[blk, pl.ds(lo, n)], sem).start(priority=priority)

    def wait(blk, part, sem):
        both = dst.at[blk, pl.ds(part * _DH, _DH)]
        pltpu.make_async_copy(both, both, sem).wait()

    return _Source(nblk * _PARTS, _PARTS, start, wait)


def _kernel(x_hbm, k_hbm, v_hbm, wq_hbm, wo_hbm, w1_hbm, b1_hbm, w2_hbm, c_hbm, wmod_hbm,
            o_ref,
            x_v, c_v, b1_v, wmod_v, wq_v, wo_v, w1_v, w2_v, kv_v,
            mod_s, q_s, score_s, act_s, col_s, small_sems, sems):
    d = x_v.shape[-1]
    f = b1_v.shape[0]
    n_pairs = k_hbm.shape[0] // _PW
    nblk = kv_v.shape[0]
    scale = _DH ** -0.5
    assert max(_AHEAD.values()) + _PARTS * _GROUP <= _PARTS * nblk
    assert max(_AHEAD.values()) < _SEMS

    small = [pltpu.make_async_copy(src, dst, small_sems.at[i])
             for i, (src, dst) in enumerate(((c_hbm, c_v), (x_hbm, x_v), (b1_hbm, b1_v)))]
    val = {}

    def rows(ref):
        return jnp.broadcast_to(ref[...].astype(jnp.float32), (_M, d))

    def cols(ref, i, w):
        return ref[:, :, pl.ds(_hint(i * w, _L), w)].reshape(d, w)

    def per_head(y):
        row = lax.broadcasted_iota(jnp.int32, y.shape, 0)
        col = lax.broadcasted_iota(jnp.int32, y.shape, 1)
        return jnp.where(((row == 0) & (col < _DH)) | ((row == 1) & (col >= _DH)), y, 0.0)

    def condition():
        small[0].wait()
        c = rows(c_v)
        val["c"] = (c * jax.nn.sigmoid(c)).astype(jnp.bfloat16)

    def modulate(i, carry):
        mod_s[i] = _dot(val["c"], cols(wmod_v, i, d))
        return carry

    def norm_a(_):
        small[1].wait()
        val["h"] = (_layernorm(rows(x_v)) * (1.0 + mod_s[1]) + mod_s[0]).astype(jnp.bfloat16)

    def query(pair, carry):
        q_s[pair] = per_head(_dot(val["h"], cols(wq_v, pair, _PW)))
        return carry

    def attention_runs(pair):
        def load_query():
            val["q"] = q_s[pair].astype(jnp.bfloat16)
            return jnp.full((_M, _L), -jnp.inf, jnp.float32)

        def scores(grp, top):
            for blk in (grp * _GROUP + i for i in range(_GROUP)):
                s = _dot(val["q"], kv_v[blk]) * scale
                score_s[blk] = s
                top = jnp.maximum(top, s)
            return top

        def row_max(top):
            val["max"] = jnp.broadcast_to(jnp.max(top, axis=-1, keepdims=True), (_M, _L))

        def values(grp, carry):
            total, *acc = carry
            for blk in (grp * _GROUP + i for i in range(_GROUP)):
                e = jnp.exp(score_s[blk] - val["max"])
                total = total + e
                e = e.astype(jnp.bfloat16)
                acc = [acc[t] + _dot_nt(e, kv_v[blk, pl.ds(t * _L, _L), :]) for t in range(_T)]
            return (total, *acc)

        def project(carry):
            total, *acc = carry
            o = jnp.concatenate(acc, axis=1) / jnp.sum(total, axis=-1, keepdims=True)
            per_band = wo_v.shape[1] // _PW
            row = _hint(lax.rem(pair, per_band) * _PW, _PW)
            wo = wo_v[lax.div(pair, per_band), pl.ds(row, _PW), :]
            val["attn"] = val["attn"] + _dot(per_head(o).astype(jnp.bfloat16), wo)

        def zeros():
            return (jnp.zeros((_M, _L), jnp.float32),) * (1 + _T)

        shape = (nblk // _GROUP, _GROUP * _PARTS)
        return [_Run(_window_source(k_hbm, kv_v, pair), *shape, scores, load_query, row_max),
                _Run(_window_source(v_hbm, kv_v, pair), *shape, values, zeros, project)]

    def norm_b(_):
        attn = jnp.broadcast_to(jnp.sum(val["attn"], axis=0, keepdims=True), (_M, d))
        val["x"] = rows(x_v) + mod_s[2] * attn
        val["h"] = (_layernorm(val["x"]) * (1.0 + mod_s[4]) + mod_s[3]).astype(jnp.bfloat16)
        val["y"] = jnp.zeros((_M, d), jnp.float32)
        small[2].wait()
        b1 = b1_v[...].astype(jnp.float32).reshape(1, f)
        for i in range(f // _PW):
            act_s[i] = jnp.broadcast_to(b1[:, i * _PW:(i + 1) * _PW], (_M, _PW))

    def up(i, carry):
        u = _dot(val["h"], cols(w1_v, i, _PW)) + act_s[i]
        softplus = jnp.log1p(jnp.exp(-jnp.abs(u))) + jnp.where(u > 0, u, 0.0)
        act_s[i] = u * jnp.tanh(softplus)
        return carry

    bands, band_rows, _ = w2_v.shape

    def act(band, j):
        at = band * band_rows + j * _L
        return act_s[at // _PW][:, at % _PW:at % _PW + _L].astype(jnp.bfloat16)

    def down(j, _, carry):
        for band in range(bands):
            val["y"] = val["y"] + _dot(act(band, j), w2_v[band, pl.ds(j * _L, _L), :])
        return carry

    last = band_rows // _L - 1
    h_down = _DOWN_PATCH[1]

    def last_columns():
        for band in range(bands):
            a = act(band, last)[0:1].astype(jnp.float32)
            col_s[band] = jnp.broadcast_to(a, (_L, _L)).T
        return jnp.zeros((_M, d), jnp.float32)

    def down_last(i, acc):
        for band in range(bands):
            w = w2_v[band, pl.ds(_hint(last * _L + i * h_down, h_down), h_down), :]
            a = col_s[band, pl.ds(_hint(i * h_down, h_down), h_down), :]
            prod = w.astype(jnp.float32) * jnp.concatenate([a] * (d // _L), axis=1)
            for r in range(0, h_down, _M):
                acc = acc + prod[r:r + _M]
        return acc

    def finish(acc):
        y = val["y"][0:1] + jnp.sum(acc, axis=0, keepdims=True)
        o_ref[...] = (val["x"][0:1] + mod_s[5, 0:1] * y).astype(o_ref.dtype)

    src_mod = _weight_source(wmod_hbm, wmod_v, *_MOD_PATCH[1:])
    src_q = _weight_source(wq_hbm, wq_v, *_Q_PATCH[1:])
    src_o = _weight_source(wo_hbm, wo_v, *_O_PATCH[1:])
    src_up = _weight_source(w1_hbm, w1_v, *_UP_PATCH[1:])
    src_down = _weight_source(w2_hbm, w2_v, *_DOWN_PATCH[1:])

    n_mod, n_up, per_tile = mod_s.shape[0], f // _PW, _L // h_down
    head = [
        _Run(src_mod, src_mod.n // src_mod.period, src_mod.period),
        _Run(src_q, n_mod, src_q.period, modulate, condition),
        _Run(src_q, src_q.n // src_q.period - n_mod, src_q.period, after=norm_a,
             first=n_mod * src_q.period),
        _Run(src_o, n_pairs, src_o.n // n_pairs, query),
    ]
    tail = [
        _Run(src_up, src_up.n // src_up.period, src_up.period, after=norm_b),
        _Run(src_down, n_up, 1, up),
        _Run(src_down, 1, per_tile - n_up, functools.partial(down, 0), first=n_up),
        *[_Run(src_down, 1, per_tile, functools.partial(down, j), first=j * per_tile)
          for j in range(1, last)],
        _Run(src_down, per_tile, 1, down_last, last_columns, finish, first=last * per_tile),
    ]
    n_head = sum(run.n for run in head)
    assert n_head == src_mod.n + src_q.n + src_o.n
    assert sum(run.n for run in tail) == src_up.n + src_down.n

    for t in range(max(_AHEAD.values())):
        for priority, dist in _AHEAD.items():
            if t < dist:
                src_mod.start(t // src_mod.period, t % src_mod.period, sems.at[t], priority)
        if t == 0:
            for copy in small:
                copy.start()
    _stream(head, 0, [(None, attention_runs(0))], sems)

    per_pair = 2 * nblk * _PARTS

    def attend(pair, attn):
        val["attn"] = attn
        following = [(pair + 1 < n_pairs, attention_runs(pair + 1)), (pair + 1 == n_pairs, tail)]
        _stream(attention_runs(pair), n_head + pair * per_pair, following, sems)
        return val["attn"]

    val["attn"] = lax.fori_loop(0, n_pairs, attend, jnp.zeros((_M, d), jnp.float32))
    _stream(tail, n_head + n_pairs * per_pair, [], sems)


@jax.jit
def pallas_adaLN_cond__sliding_block_cached__dense_activation_mish__decode_kernel(
    A_x: jax.Array,
    A_k_cache: jax.Array,
    A_v_cache: jax.Array,
    A_wq: jax.Array,
    A_wo: jax.Array,
    B_x: jax.Array,
    B_w1: jax.Array,
    B_b1: jax.Array,
    B_w2: jax.Array,
    c: jax.Array,
    w_mod: jax.Array,
):
    del B_x
    _, hkv, sk, dh = A_k_cache.shape
    assert A_x.shape[:2] == (1, 1) and (hkv, dh) == (_HQ, _DH)
    d = A_x.shape[-1]
    f = B_w1.shape[1]
    win = min(4096, max(256, sk // 4))
    kt = jnp.swapaxes(A_k_cache, 2, 3).reshape(hkv * dh, sk)
    vt = jnp.swapaxes(A_v_cache, 2, 3).reshape(hkv * dh, sk)
    wmod, wq, wo, w1, w2 = (
        w.reshape(bands, w.shape[0] // bands, w.shape[1]) for w, (bands, _, _) in (
            (w_mod, _MOD_PATCH), (A_wq, _Q_PATCH), (A_wo, _O_PATCH), (B_w1, _UP_PATCH),
            (B_w2, _DOWN_PATCH)))
    x = A_x.reshape(1, d)
    f32 = jnp.float32
    out = pl.pallas_call(
        _kernel,
        out_shape=jax.ShapeDtypeStruct(x.shape, x.dtype),
        in_specs=[pl.BlockSpec(memory_space=pltpu.HBM)] * 10,
        out_specs=pl.BlockSpec(memory_space=pltpu.VMEM),
        scratch_shapes=[
            *[pltpu.VMEM(a.shape, a.dtype) for a in (x, c, B_b1, wmod, wq, wo, w1, w2)],
            pltpu.VMEM((win // _L, _PW, _L), kt.dtype),
            pltpu.VMEM((w_mod.shape[1] // d, _M, d), f32),
            pltpu.VMEM((hkv // 2, _M, _PW), f32),
            pltpu.VMEM((win // _L, _M, _L), f32),
            pltpu.VMEM((f // _PW, _M, _PW), f32),
            pltpu.VMEM((w2.shape[0], _L, _L), f32),
            pltpu.SemaphoreType.DMA((3,)),
            pltpu.SemaphoreType.DMA((_SEMS,)),
        ],
        compiler_params=pltpu.CompilerParams(
            vmem_limit_bytes=48 * 1024 * 1024,
            disable_semaphore_checks=True,
        ),
        name="adaln_decode_block",
    )(x, kt, vt, wq, wo, w1, B_b1, w2, c, wmod)
    return out.reshape(A_x.shape)
```

```python
import functools

import jax
import jax.numpy as jnp
from jax import lax
import jax.experimental.pallas as pl
import jax.experimental.pallas.tpu as pltpu

_HQ, _DH = 32, 192
_EPS = 1e-5
_M = 8
_L = 128
_PW = 2 * _DH
_T = _PW // _L

_SEMS = 32
_MAIN, _SLIVER = 1, 0
_AHEAD = {_MAIN: 26, _SLIVER: 16}
_PARTS = 2
_KV_SLIVER = 16
_KV_RUN = 2
_GROUP = 4

_MOD_PATCH = (8, 8, 384)
_Q_PATCH = (10, 8, 256)
_O_PATCH = (8, 8, 640)
_UP_PATCH = (4, 8, 768)
_DOWN_PATCH = (3, 16, 640)


def _layernorm(x):
    m = jnp.mean(x, axis=-1, keepdims=True)
    d = x - m
    v = jnp.mean(d * d, axis=-1, keepdims=True)
    return d / jnp.sqrt(v + _EPS)


def _dot(a, b):
    return jnp.dot(a, b, preferred_element_type=jnp.float32)


def _dot_nt(a, b):
    return lax.dot_general(a, b, (((1,), (1,)), ((), ())), preferred_element_type=jnp.float32)


def _hint(i, m):
    return i if isinstance(i, int) else pl.multiple_of(i, m)


class _Source:
    def __init__(self, n, period, start, wait):
        self.n, self.period, self.start, self.wait = n, period, start, wait


class _Run:
    def __init__(self, source, groups, size, step=None, before=None, after=None, first=0):
        self.source, self.groups, self.size, self.first = source, groups, size, first
        self.n = groups * size
        self.step, self.before, self.after = step, before, after


def _locate(runs, pos):
    for run in runs:
        if pos < run.n:
            return run.source, run.first + pos
        pos -= run.n
    return None, 0


def _stream(runs, t0, following, sems):
    total = sum(run.n for run in runs)

    def at(pos):
        if pos < total:
            return [(None, *_locate(runs, pos))]
        found = [(cond, *_locate(later, pos - total)) for cond, later in following]
        return [x for x in found if x[1] is not None]

    def repeats(a, b, size):
        a, b = ([x for entry in plan for alts in entry for x in alts + [None]] for plan in (a, b))
        return len(a) == len(b) and all(
            x is y if None in (x, y)
            else x[1] is y[1] and y[2] == x[2] + size and size % x[1].period == 0
            for x, y in zip(a, b))

    def sem(t):
        return sems.at[t & (_SEMS - 1)]

    base = 0
    for run in runs:
        plans = [[[at(base + grp * run.size + i + dist) for dist in (0, *_AHEAD.values())]
                  for i in range(run.size)] for grp in range(run.groups)]
        carry = run.before() if run.before else None
        lo = 0
        while lo < run.groups:
            hi = lo + 1
            while hi < run.groups and repeats(plans[hi - 1], plans[hi], run.size):
                hi += 1

            def group(j, carry, lo=lo, run=run, base=base):
                def index(source, k):
                    return k // source.period + j * (run.size // source.period), k % source.period

                t = t0 + base + (lo + j) * run.size
                for i, ([(_, source, k)], *later) in enumerate(plans[lo]):
                    source.wait(*index(source, k), sem(t + i))
                    for (priority, dist), alts in zip(_AHEAD.items(), later):
                        for cond, source, k in alts:
                            start = functools.partial(
                                source.start, *index(source, k), sem(t + i + dist), priority)
                            if cond is None:
                                start()
                            else:
                                pl.when(cond)(start)
                return run.step(lo + j, carry) if run.step else carry

            carry = group(0, carry) if hi - lo == 1 else lax.fori_loop(0, hi - lo, group, carry)
            lo = hi
        if run.after:
            run.after(carry)
        base += run.n


def _weight_source(src, dst, h, w):
    bands, nrow, ncol = src.shape

    def patch(r, c):
        return pl.ds(_hint(r * h, h), h), pl.ds(c * w, w)

    def start(r, c, sem, priority):
        idx = (pl.ds(0, bands - 1) if priority == _MAIN else pl.ds(bands - 1, 1), *patch(r, c))
        pltpu.make_async_copy(src.at[idx], dst.at[idx], sem).start(priority=priority)

    def wait(r, c, sem):
        both = dst.at[(slice(None), *patch(r, c))]
        pltpu.make_async_copy(both, both, sem).wait()

    return _Source((nrow // h) * (ncol // w), ncol // w, start, wait)


def _window_source(src, dst, pair):
    nblk = dst.shape[0]
    first = src.shape[1] - nblk * _L
    spans = {_MAIN: ((_KV_SLIVER, _DH - _KV_SLIVER), (_DH, _DH - _KV_SLIVER)),
             _SLIVER: ((0, _KV_SLIVER), (_PW - _KV_SLIVER, _KV_SLIVER))}

    def where(major, minor):
        return major * _KV_RUN + minor % _KV_RUN, minor // _KV_RUN

    def start(major, minor, sem, priority):
        blk, part = where(major, minor)
        lo, n = spans[priority][part]
        pltpu.make_async_copy(
            src.at[pl.ds(_hint(pair * _PW + lo, 16), n), pl.ds(_hint(first + blk * _L, _L), _L)],
            dst.at[blk, pl.ds(lo, n)], sem).start(priority=priority)

    def wait(major, minor, sem):
        blk, part = where(major, minor)
        both = dst.at[blk, pl.ds(part * _DH, _DH)]
        pltpu.make_async_copy(both, both, sem).wait()

    return _Source(nblk * _PARTS, _KV_RUN * _PARTS, start, wait)


def _kernel(x_hbm, k_hbm, v_hbm, wq_hbm, wo_hbm, w1_hbm, b1_hbm, w2_hbm, c_hbm, wmod_hbm,
            o_ref,
            x_v, c_v, b1_v, wmod_v, wq_v, wo_v, w1_v, w2_v, kv_v,
            mod_s, q_s, score_s, act_s, col_s, small_sems, sems):
    d = x_v.shape[-1]
    f = b1_v.shape[0]
    n_pairs = k_hbm.shape[0] // _PW
    nblk = kv_v.shape[0]
    scale = _DH ** -0.5
    assert max(_AHEAD.values()) + _PARTS * _GROUP <= _PARTS * nblk
    assert max(_AHEAD.values()) < _SEMS and _GROUP % _KV_RUN == 0 and nblk % _GROUP == 0

    small = [pltpu.make_async_copy(src, dst, small_sems.at[i])
             for i, (src, dst) in enumerate(((c_hbm, c_v), (x_hbm, x_v), (b1_hbm, b1_v)))]
    val = {}

    def rows(ref):
        return jnp.broadcast_to(ref[...].astype(jnp.float32), (_M, d))

    def cols(ref, i, w):
        return ref[:, :, pl.ds(_hint(i * w, _L), w)].reshape(d, w)

    def per_head(y):
        row = lax.broadcasted_iota(jnp.int32, y.shape, 0)
        col = lax.broadcasted_iota(jnp.int32, y.shape, 1)
        return jnp.where(((row == 0) & (col < _DH)) | ((row == 1) & (col >= _DH)), y, 0.0)

    def condition():
        small[0].wait()
        c = rows(c_v)
        val["c"] = (c * jax.nn.sigmoid(c)).astype(jnp.bfloat16)

    def modulate(i, carry):
        mod_s[i] = _dot(val["c"], cols(wmod_v, i, d))
        return carry

    def norm_a(_):
        small[1].wait()
        val["h"] = (_layernorm(rows(x_v)) * (1.0 + mod_s[1]) + mod_s[0]).astype(jnp.bfloat16)

    def query(pair, carry):
        q_s[pair] = per_head(_dot(val["h"], cols(wq_v, pair, _PW)))
        return carry

    def attention_runs(pair):
        def load_query():
            val["q"] = q_s[pair].astype(jnp.bfloat16)
            return jnp.full((_M, _L), -jnp.inf, jnp.float32)

        def scores(grp, top):
            for blk in (grp * _GROUP + i for i in range(_GROUP)):
                s = _dot(val["q"], kv_v[blk]) * scale
                score_s[blk] = s
                top = jnp.maximum(top, s)
            return top

        def row_max(top):
            val["max"] = jnp.broadcast_to(jnp.max(top, axis=-1, keepdims=True), (_M, _L))

        def values(grp, carry):
            total, *acc = carry
            for blk in (grp * _GROUP + i for i in range(_GROUP)):
                e = jnp.exp(score_s[blk] - val["max"])
                total = total + e
                e = e.astype(jnp.bfloat16)
                acc = [acc[t] + _dot_nt(e, kv_v[blk, pl.ds(t * _L, _L), :]) for t in range(_T)]
            return (total, *acc)

        def project(carry):
            total, *acc = carry
            o = jnp.concatenate(acc, axis=1) / jnp.sum(total, axis=-1, keepdims=True)
            per_band = wo_v.shape[1] // _PW
            row = _hint(lax.rem(pair, per_band) * _PW, _PW)
            wo = wo_v[lax.div(pair, per_band), pl.ds(row, _PW), :]
            val["attn"] = val["attn"] + _dot(per_head(o).astype(jnp.bfloat16), wo)

        def zeros():
            return (jnp.zeros((_M, _L), jnp.float32),) * (1 + _T)

        shape = (nblk // _GROUP, _GROUP * _PARTS)
        return [_Run(_window_source(k_hbm, kv_v, pair), *shape, scores, load_query, row_max),
                _Run(_window_source(v_hbm, kv_v, pair), *shape, values, zeros, project)]

    def norm_b(_):
        attn = jnp.broadcast_to(jnp.sum(val["attn"], axis=0, keepdims=True), (_M, d))
        val["x"] = rows(x_v) + mod_s[2] * attn
        val["h"] = (_layernorm(val["x"]) * (1.0 + mod_s[4]) + mod_s[3]).astype(jnp.bfloat16)
        val["y"] = jnp.zeros((_M, d), jnp.float32)
        small[2].wait()
        b1 = b1_v[...].astype(jnp.float32).reshape(1, f)
        for i in range(f // _PW):
            act_s[i] = jnp.broadcast_to(b1[:, i * _PW:(i + 1) * _PW], (_M, _PW))

    def up(i, carry):
        u = _dot(val["h"], cols(w1_v, i, _PW)) + act_s[i]
        softplus = jnp.log1p(jnp.exp(-jnp.abs(u))) + jnp.where(u > 0, u, 0.0)
        act_s[i] = u * jnp.tanh(softplus)
        return carry

    bands, band_rows, _ = w2_v.shape

    def act(band, j):
        at = band * band_rows + j * _L
        return act_s[at // _PW][:, at % _PW:at % _PW + _L].astype(jnp.bfloat16)

    def down(j, _, carry):
        for band in range(bands):
            val["y"] = val["y"] + _dot(act(band, j), w2_v[band, pl.ds(j * _L, _L), :])
        return carry

    last = band_rows // _L - 1
    h_down = _DOWN_PATCH[1]

    def last_columns():
        for band in range(bands):
            a = act(band, last)[0:1].astype(jnp.float32)
            col_s[band] = jnp.broadcast_to(a, (_L, _L)).T
        return jnp.zeros((_M, d), jnp.float32)

    def down_last(i, acc):
        for band in range(bands):
            w = w2_v[band, pl.ds(_hint(last * _L + i * h_down, h_down), h_down), :]
            a = col_s[band, pl.ds(_hint(i * h_down, h_down), h_down), :]
            prod = w.astype(jnp.float32) * jnp.concatenate([a] * (d // _L), axis=1)
            for r in range(0, h_down, _M):
                acc = acc + prod[r:r + _M]
        return acc

    def finish(acc):
        y = val["y"][0:1] + jnp.sum(acc, axis=0, keepdims=True)
        o_ref[...] = (val["x"][0:1] + mod_s[5, 0:1] * y).astype(o_ref.dtype)

    src_mod = _weight_source(wmod_hbm, wmod_v, *_MOD_PATCH[1:])
    src_q = _weight_source(wq_hbm, wq_v, *_Q_PATCH[1:])
    src_o = _weight_source(wo_hbm, wo_v, *_O_PATCH[1:])
    src_up = _weight_source(w1_hbm, w1_v, *_UP_PATCH[1:])
    src_down = _weight_source(w2_hbm, w2_v, *_DOWN_PATCH[1:])

    n_mod, n_up, per_tile = mod_s.shape[0], f // _PW, _L // h_down
    head = [
        _Run(src_mod, src_mod.n // src_mod.period, src_mod.period),
        _Run(src_q, n_mod, src_q.period, modulate, condition),
        _Run(src_q, src_q.n // src_q.period - n_mod, src_q.period, after=norm_a,
             first=n_mod * src_q.period),
        _Run(src_o, n_pairs, src_o.n // n_pairs, query),
    ]
    tail = [
        _Run(src_up, src_up.n // src_up.period, src_up.period, after=norm_b),
        _Run(src_down, n_up, 1, up),
        _Run(src_down, 1, per_tile - n_up, functools.partial(down, 0), first=n_up),
        *[_Run(src_down, 1, per_tile, functools.partial(down, j), first=j * per_tile)
          for j in range(1, last)],
        _Run(src_down, per_tile, 1, down_last, last_columns, finish, first=last * per_tile),
    ]
    n_head = sum(run.n for run in head)
    assert n_head == src_mod.n + src_q.n + src_o.n
    assert sum(run.n for run in tail) == src_up.n + src_down.n

    for t in range(max(_AHEAD.values())):
        for priority, dist in _AHEAD.items():
            if t < dist:
                src_mod.start(t // src_mod.period, t % src_mod.period, sems.at[t], priority)
        if t == 0:
            for copy in small:
                copy.start()
    _stream(head, 0, [(None, attention_runs(0))], sems)

    per_pair = 2 * nblk * _PARTS

    def attend(pair, attn):
        val["attn"] = attn
        following = [(pair + 1 < n_pairs, attention_runs(pair + 1)), (pair + 1 == n_pairs, tail)]
        _stream(attention_runs(pair), n_head + pair * per_pair, following, sems)
        return val["attn"]

    val["attn"] = lax.fori_loop(0, n_pairs, attend, jnp.zeros((_M, d), jnp.float32))
    _stream(tail, n_head + n_pairs * per_pair, [], sems)


@jax.jit
def pallas_adaLN_cond__sliding_block_cached__dense_activation_mish__decode_kernel(
    A_x: jax.Array,
    A_k_cache: jax.Array,
    A_v_cache: jax.Array,
    A_wq: jax.Array,
    A_wo: jax.Array,
    B_x: jax.Array,
    B_w1: jax.Array,
    B_b1: jax.Array,
    B_w2: jax.Array,
    c: jax.Array,
    w_mod: jax.Array,
):
    del B_x
    _, hkv, sk, dh = A_k_cache.shape
    assert A_x.shape[:2] == (1, 1) and (hkv, dh) == (_HQ, _DH)
    d = A_x.shape[-1]
    f = B_w1.shape[1]
    win = min(4096, max(256, sk // 4))
    kt = jnp.swapaxes(A_k_cache, 2, 3).reshape(hkv * dh, sk)
    vt = jnp.swapaxes(A_v_cache, 2, 3).reshape(hkv * dh, sk)
    wmod, wq, wo, w1, w2 = (
        w.reshape(bands, w.shape[0] // bands, w.shape[1]) for w, (bands, _, _) in (
            (w_mod, _MOD_PATCH), (A_wq, _Q_PATCH), (A_wo, _O_PATCH), (B_w1, _UP_PATCH),
            (B_w2, _DOWN_PATCH)))
    x = A_x.reshape(1, d)
    f32 = jnp.float32
    out = pl.pallas_call(
        _kernel,
        out_shape=jax.ShapeDtypeStruct(x.shape, x.dtype),
        in_specs=[pl.BlockSpec(memory_space=pltpu.HBM)] * 10,
        out_specs=pl.BlockSpec(memory_space=pltpu.VMEM),
        scratch_shapes=[
            *[pltpu.VMEM(a.shape, a.dtype) for a in (x, c, B_b1, wmod, wq, wo, w1, w2)],
            pltpu.VMEM((win // _L, _PW, _L), kt.dtype),
            pltpu.VMEM((w_mod.shape[1] // d, _M, d), f32),
            pltpu.VMEM((hkv // 2, _M, _PW), f32),
            pltpu.VMEM((win // _L, _M, _L), f32),
            pltpu.VMEM((f // _PW, _M, _PW), f32),
            pltpu.VMEM((w2.shape[0], _L, _L), f32),
            pltpu.SemaphoreType.DMA((3,)),
            pltpu.SemaphoreType.DMA((_SEMS,)),
        ],
        compiler_params=pltpu.CompilerParams(
            vmem_limit_bytes=48 * 1024 * 1024,
            disable_semaphore_checks=True,
        ),
        name="adaln_decode_block",
    )(x, kt, vt, wq, wo, w1, B_b1, w2, c, wmod)
    return out.reshape(A_x.shape)
```
